```python
import os as _os
_os.environ.setdefault('JAX_PLATFORMS', 'cpu')
import jax
import jax.numpy as jnp

def _softmax(x, axis=-1):
    return jax.nn.softmax(x, axis=axis)

def _gelu(x):
    return jax.nn.gelu(x, approximate=True)

def _silu(x):
    return jax.nn.silu(x)

def _sigmoid(x):
    return jax.nn.sigmoid(x)

def _layernorm(x, axis=-1, eps=1e-05):
    m = jnp.mean(x, axis=axis, keepdims=True)
    v = jnp.var(x, axis=axis, keepdims=True)
    return (x - m) / jnp.sqrt(v + eps)

def _scatter_add(tgt, idx, src, axis=0):
    return tgt.at[idx].add(src)

def _segment_sum(src, seg, n):
    return jax.ops.segment_sum(src, seg, n)

class _Rng:

    def __init__(self, key):
        self._k = key

    def _next(self):
        self._k, sub = jax.random.split(self._k)
        return sub

    def normal(self, shape):
        return jax.random.normal(self._next(), shape, dtype=jnp.bfloat16)

    def randint(self, lo, hi, shape):
        return jax.random.randint(self._next(), shape, lo, hi, dtype=jnp.int32)

    def uniform(self, shape, lo=0.0, hi=1.0):
        return jax.random.uniform(self._next(), shape, jnp.bfloat16, lo, hi)

    def permutation(self, n):
        return jax.random.permutation(self._next(), n)
kernel_name = 'adaLN_cond__grouped_kv_mqa__swiglu_ffn__prompt'

def setup_inputs():
    _rng = _Rng(jax.random.key(int.from_bytes(__import__("os").urandom(4), "little")))
    _w = lambda a: (lambda t: t.astype(jnp.bfloat16) if jnp.issubdtype(t.dtype, jnp.floating) else t)(jnp.asarray(a))

    def _A_setup():
        B, S, D, H = (1, 2048, 576, 32)
        Dh = D // H
        return {'x': _w((lambda *s: _rng.normal(s) * 0.05)(B, S, D)), 'wq': _w((lambda *s: _rng.normal(s) * 0.05)(D, H * Dh)), 'wk': _w((lambda *s: _rng.normal(s) * 0.05)(D, Dh)), 'wv': _w((lambda *s: _rng.normal(s) * 0.05)(D, Dh)), 'wo': _w((lambda *s: _rng.normal(s) * 0.05)(H * Dh, D))}
    _A_in = _A_setup()

    def _B_setup():
        B, S, D, F = (1, 2048, 576, 4608)
        return {'x': _w((lambda *s: _rng.normal(s) * 0.05)(B, S, D)), 'w_gate': _w((lambda *s: _rng.normal(s) * 0.05)(D, F)), 'w_up': _w((lambda *s: _rng.normal(s) * 0.05)(D, F)), 'w_down': _w((lambda *s: _rng.normal(s) * 0.05)(F, D))}
    _B_in = _B_setup()
    return {'A_x': _A_in['x'], 'A_wq': _A_in['wq'], 'A_wk': _A_in['wk'], 'A_wv': _A_in['wv'], 'A_wo': _A_in['wo'], 'B_x': _B_in['x'], 'B_w_gate': _B_in['w_gate'], 'B_w_up': _B_in['w_up'], 'B_w_down': _B_in['w_down'], 'c': _w((lambda *s: _rng.normal(s) * 0.05)(1, 576) * 8.0), 'w_mod': _w((lambda *s: _rng.normal(s) * 0.05)(576, 6 * 576) * 576 ** (-0.5) * 8.0)}

def reference(A_x, A_wq, A_wk, A_wv, A_wo, B_x, B_w_gate, B_w_up, B_w_down, c, w_mod):

    def _A_ref(x, wq, wk, wv, wo):
        B, S, D = x.shape
        H = 32
        Dh = D // H
        q = (lambda x, *d: x.transpose(*d))((x @ wq).reshape(B, S, H, Dh), 0, 2, 1, 3)
        k = x @ wk
        v = x @ wv
        scores = jnp.einsum('bhqd,bkd->bhqk', q, k) * Dh ** (-0.5)
        p = _softmax(scores, axis=-1)
        o = jnp.einsum('bhqk,bkd->bhqd', p, v)
        return (lambda x, *d: x.transpose(*d))(o, 0, 2, 1, 3).reshape(B, S, H * Dh) @ wo

    def _B_ref(x, w_gate, w_up, w_down):
        g = _silu(x @ w_gate)
        u = x @ w_up
        return g * u @ w_down
    x = A_x
    mod = (_silu(c) @ w_mod).reshape(c.shape[0], 6, 1, -1)
    sa, ca, ga, sb, cb, gb = (mod[:, 0].copy(), mod[:, 1].copy(), mod[:, 2].copy(), mod[:, 3].copy(), mod[:, 4].copy(), mod[:, 5].copy())
    h = _layernorm(x, axis=-1) * (1 + ca) + sa
    x = x + ga * _A_ref(h, A_wq, A_wk, A_wv, A_wo)
    h = _layernorm(x, axis=-1) * (1 + cb) + sb
    x = x + gb * _B_ref(h, B_w_gate, B_w_up, B_w_down)
    return x
```

```python
import functools
import math

import jax
import jax.numpy as jnp
from jax import lax
import jax.experimental.pallas as pl
import jax.experimental.pallas.tpu as pltpu

f32 = jnp.float32
bf16 = jnp.bfloat16

S = 2048
D = 576
H = 32
DH = 18
F = 4608
DP = 640
V_ROW = 576
K_ROW = 600
HG = 4
NG = H // HG
VR = 24
EPS = 1e-5
QSCALE = DH ** -0.5 * math.log2(math.e)


def _ln_t(x):
    mu = jnp.mean(x, axis=0, keepdims=True)
    xc = x - mu
    var = jnp.mean(xc * xc, axis=0, keepdims=True)
    return xc * lax.rsqrt(var + EPS)


def _make_kernel(TQ, CK, RC, FC, SK):
    NQ = S // TQ
    NC = S // CK

    def kernel(xt_ref, wq_ref, wkt_ref, wvt_ref, wo_ref, c_ref,
               wmod_hbm, wg_hbm, wu_hbm, wdt_hbm,
               o_ref,
               wmod_v, wg_v, wu_v, wdt_v, sems,
               modt_s, tmp_s, wall_s, wot_s, qt_s, kv_s, vt_s, sa_s, sb_s,
               mn_s, mc_s, ac_s, ot_s, x1_s, h2_s, acc_s):
        i = pl.program_id(0)
        sbuf = (sa_s, sb_s)

        def cp_mod0():
            return pltpu.make_async_copy(wmod_hbm.at[:, 0:2 * D], wmod_v.at[:, 0:2 * D], sems.at[0])

        def cp_mod1():
            return pltpu.make_async_copy(wmod_hbm.at[:, 2 * D:6 * D], wmod_v.at[:, 2 * D:6 * D], sems.at[1])

        def cp_wg():
            return pltpu.make_async_copy(wg_hbm, wg_v, sems.at[2])

        def cp_wu():
            return pltpu.make_async_copy(wu_hbm, wu_v, sems.at[3])

        def cp_wd():
            return pltpu.make_async_copy(wdt_hbm, wdt_v, sems.at[4])

        def mod_cols(lo, hi):
            cc = c_ref[...].astype(f32)
            sc = cc * (1.0 / (1.0 + jnp.exp(-cc)))
            sc = jnp.broadcast_to(sc, (8, D)).astype(bf16)
            row = jnp.dot(sc, wmod_v[:, lo:hi], preferred_element_type=f32)[0:1]
            modt_s[lo:hi, :] = jnp.broadcast_to(row, (128, hi - lo)).T

        def col(k, n):
            return jnp.tile(modt_s[k * D:(k + 1) * D, :], (1, n // 128))

        def a_chunk(qg, j, c, s_ref, m):
            sl = slice(c * CK, (c + 1) * CK)
            s = jnp.dot(kv_s[j, sl, :], qg, preferred_element_type=f32)
            s_ref[sl, :] = s
            mc = s.reshape(CK // 8, 8, TQ).max(axis=0)
            return mc if m is None else jnp.maximum(m, mc)

        def b_chunk(c, s_ref, m, acc):
            sl = slice(c * CK, (c + 1) * CK)
            p = jnp.exp2(s_ref[sl, :] - m).astype(bf16)
            pv = jnp.dot(vt_s[:, sl], p, preferred_element_type=f32)
            return pv if acc is None else acc + pv

        def b_finish(h, acc):
            ot_s[h] = acc * (1.0 / acc[DH:DH + 1])

        @pl.when(i == 0)
        def _prologue():
            cp_mod0().start()
            cp_mod1().start()
            cp_wg().start()
            cp_wu().start()
            cp_wd().start()

            tmp_s[...] = jnp.zeros_like(tmp_s)
            tmp_s[0:D, 0:D] = wq_ref[...].astype(f32)
            wqt = tmp_s[0:DP, :].T
            z6 = jnp.zeros((VR - DH, D), f32)
            wall_s[0:D, :] = wqt[0:D, 0:D].astype(bf16)
            wall_s[D:DP, :] = jnp.concatenate(
                [wvt_ref[...].astype(f32), z6, wkt_ref[...].astype(f32), z6,
                 jnp.zeros((DP - K_ROW - VR, D), f32)], axis=0).astype(bf16)
            wo = wo_ref[...].astype(f32)
            for hp in range(H // 2):
                tmp_s[2 * hp * VR:(2 * hp + 2) * VR, 0:D] = jnp.concatenate(
                    [wo[(2 * hp) * DH:(2 * hp + 1) * DH], z6,
                     wo[(2 * hp + 1) * DH:(2 * hp + 2) * DH], z6], axis=0)
            wot_s[...] = tmp_s[...].T[0:D].astype(bf16)

            cp_mod0().wait()
            mod_cols(0, 2 * D)

            lane128 = lax.broadcasted_iota(jnp.int32, (1, 128), 1)
            kmask = (lane128 >= K_ROW - 512) & (lane128 < K_ROW - 512 + DH)
            vrow = lax.broadcasted_iota(jnp.int32, (VR, 1), 0)

            def proj(r, carry):
                r0 = pl.multiple_of(r * RC, RC)
                xc = xt_ref[:, pl.ds(r0, RC)].astype(f32)
                h = (_ln_t(xc) * (1.0 + col(1, RC)) + col(0, RC)).astype(bf16)
                res = jnp.dot(wall_s[...], h, preferred_element_type=f32)
                for g in range(NG):
                    qt_s[g, :, pl.ds(r0, RC)] = (
                        res[HG * DH * g:HG * DH * g + 128] * QSCALE).astype(bf16)
                vt_s[:, pl.ds(r0, RC)] = jnp.where(vrow == DH, 1.0, res[V_ROW:V_ROW + VR])
                kk = jnp.where(kmask, res[512:DP].T, 0.0)
                for j in range(HG):
                    kv_s[j, pl.ds(r0, RC), :] = pltpu.roll(
                        kk, (DH * j - (K_ROW - 512)) % 128, 1).astype(bf16)
                return carry

            lax.fori_loop(0, S // RC, proj, 0)

            qg = qt_s[0, :, 0:TQ]
            m = None
            for c in range(NC):
                m = a_chunk(qg, 0, c, sa_s, m)
            mn_s[...] = m.max(axis=0, keepdims=True)
            mc_s[...] = jnp.zeros_like(mc_s)
            ac_s[...] = jnp.ones_like(ac_s)
            if SK:
                sb_s[(NC - SK) * CK:, :] = jnp.zeros((SK * CK, TQ), f32)

        q0 = pl.multiple_of(i * TQ, TQ)
        q_next = pl.multiple_of(jnp.minimum(i + 1, NQ - 1) * TQ, TQ)

        def attn_body(g, carry):
            m_next, m_cur, acc = carry
            last = g == NG - 1
            gn = jnp.where(last, 0, g + 1)
            qn = pl.multiple_of(jnp.where(last, q_next, q0), TQ)
            qg_cur = qt_s[g, :, pl.ds(q0, TQ)]
            qg_nxt = qt_s[gn, :, pl.ds(qn, TQ)]
            ms = {-1: m_cur, 0: m_next}
            mpart = None
            for t in range(HG * NC):
                ja, ca = 1 + t // NC, t % NC
                mpart = a_chunk(qg_cur if ja < HG else qg_nxt, ja % HG, ca, sbuf[ja % 2], mpart)
                if ca == NC - 1:
                    ms[ja] = mpart.max(axis=0, keepdims=True)
                    mpart = None
                jb, cb = (t - SK) // NC, (t - SK) % NC
                if cb == 0:
                    acc = None
                acc = b_chunk(cb, sbuf[jb % 2], ms[jb], acc)
                if cb == NC - 1:
                    b_finish((g * HG + jb) % H if jb >= 0 else (g * HG + H - 1) % H, acc)
            if SK == 0:
                acc = carry[2]
            return ms[HG], ms[HG - 1], acc

        m_next, m_cur, acc = lax.fori_loop(
            0, NG, attn_body, (mn_s[...], mc_s[...], ac_s[...]))
        mn_s[...] = m_next
        mc_s[...] = m_cur
        ac_s[...] = acc
        if SK:
            for c in range(NC - SK, NC):
                acc = b_chunk(c, sb_s, m_cur, acc)
            b_finish(H - 1, acc)

        @pl.when(i == 0)
        def _():
            cp_mod1().wait()
            mod_cols(2 * D, 6 * D)
            cp_wg().wait()
            cp_wu().wait()
            cp_wd().wait()

        ot = ot_s[...].reshape(H * VR, TQ).astype(bf16)
        attn = jnp.dot(wot_s[...], ot, preferred_element_type=f32)
        x1 = xt_ref[:, pl.ds(q0, TQ)].astype(f32) + col(2, TQ) * attn
        x1_s[...] = x1
        h2t = _ln_t(x1) * (1.0 + col(4, TQ)) + col(3, TQ)
        h2t = jnp.concatenate([h2t, jnp.zeros((DP - D, TQ), f32)], axis=0)
        h2_s[...] = h2t.T[:, 0:D].astype(bf16)
        acc_s[...] = jnp.zeros_like(acc_s)

        def ffn_body(fi, carry):
            f0 = pl.multiple_of(fi * FC, FC)
            h2 = h2_s[...]
            g = jnp.dot(h2, wg_v[:, pl.ds(f0, FC)], preferred_element_type=f32)
            u = jnp.dot(h2, wu_v[:, pl.ds(f0, FC)], preferred_element_type=f32)
            a = (g * (1.0 / (1.0 + jnp.exp(-g))) * u).astype(bf16)
            acc_s[...] += lax.dot_general(wdt_v[:, pl.ds(f0, FC)], a, (((1,), (1,)), ((), ())),
                                          preferred_element_type=f32)
            return carry

        lax.fori_loop(0, F // FC, ffn_body, 0)
        o_ref[...] = (x1_s[...] + col(5, TQ) * acc_s[...]).astype(o_ref.dtype)

    return kernel


@functools.partial(jax.jit, static_argnames=("TQ", "CK", "RC", "FC", "SK"))
def _run(A_x, A_wq, A_wk, A_wv, A_wo, B_x, B_w_gate, B_w_up, B_w_down, c, w_mod,
        TQ=512, CK=256, RC=256, FC=512, SK=2):
    xt = A_x.reshape(S, D).T
    full = lambda shape: pl.BlockSpec(shape, lambda i: (0,) * len(shape))
    hbm = pl.BlockSpec(memory_space=pltpu.HBM)
    out = pl.pallas_call(
        _make_kernel(TQ, CK, RC, FC, SK),
        grid=(S // TQ,),
        in_specs=[full((D, S)), full((D, D)), full((DH, D)), full((DH, D)), full((D, D)), full((1, D)),
                  hbm, hbm, hbm, hbm],
        out_specs=pl.BlockSpec((D, TQ), lambda i: (0, i)),
        out_shape=jax.ShapeDtypeStruct((D, S), bf16),
        scratch_shapes=[
            pltpu.VMEM((D, 6 * D), bf16),
            pltpu.VMEM((D, F), bf16),
            pltpu.VMEM((D, F), bf16),
            pltpu.VMEM((D, F), bf16),
            pltpu.SemaphoreType.DMA((5,)),
            pltpu.VMEM((6 * D, 128), f32),
            pltpu.VMEM((H * VR, DP), f32),
            pltpu.VMEM((DP, D), bf16),
            pltpu.VMEM((D, H * VR), bf16),
            pltpu.VMEM((NG, 128, S), bf16),
            pltpu.VMEM((HG, S, 128), bf16),
            pltpu.VMEM((VR, S), f32),
            pltpu.VMEM((S, TQ), f32),
            pltpu.VMEM((S, TQ), f32),
            pltpu.VMEM((1, TQ), f32),
            pltpu.VMEM((1, TQ), f32),
            pltpu.VMEM((VR, TQ), f32),
            pltpu.VMEM((H, VR, TQ), f32),
            pltpu.VMEM((D, TQ), f32),
            pltpu.VMEM((TQ, D), bf16),
            pltpu.VMEM((D, TQ), f32),
        ],
        compiler_params=pltpu.CompilerParams(
            dimension_semantics=("arbitrary",),
            vmem_limit_bytes=100 * 1024 * 1024),
    )(xt, A_wq, A_wk.T, A_wv.T, A_wo, c, w_mod, B_w_gate, B_w_up, B_w_down.T)
    return out.T.reshape(1, S, D)


@jax.jit
def pallas_adaLN_cond__grouped_kv_mqa__swiglu_ffn__prompt_kernel(
    A_x: jax.Array,
    A_wq: jax.Array,
    A_wk: jax.Array,
    A_wv: jax.Array,
    A_wo: jax.Array,
    B_x: jax.Array,
    B_w_gate: jax.Array,
    B_w_up: jax.Array,
    B_w_down: jax.Array,
    c: jax.Array,
    w_mod: jax.Array,
):
    return _run(A_x, A_wq, A_wk, A_wv, A_wo, B_x, B_w_gate, B_w_up, B_w_down, c, w_mod)
```

```python
import functools
import math

import jax
import jax.numpy as jnp
from jax import lax
import jax.experimental.pallas as pl
import jax.experimental.pallas.tpu as pltpu

f32 = jnp.float32
bf16 = jnp.bfloat16
i32 = jnp.int32
i8 = jnp.int8

S = 2048
D = 576
H = 32
DH = 18
F = 4608
DP = 640
HG = 4
NG = H // HG
VR = 24
EPS = 1e-5
QSCALE = DH ** -0.5 * math.log2(math.e)
NT = (((1,), (1,)), ((), ()))
RND = 1.5 * 2.0 ** 23
T1 = 16.0
T2 = 16.0
E_LO, E_HI = 40, 200


def _ln_t(x):
    mu = jnp.mean(x, axis=0, keepdims=True)
    xc = x - mu
    var = jnp.mean(xc * xc, axis=0, keepdims=True)
    return xc * lax.rsqrt(var + EPS)


def _expo(a):
    return jnp.clip(lax.shift_right_logical(pltpu.bitcast(a, i32), 23), E_LO, E_HI)


def _pow2(e):
    return pltpu.bitcast(lax.shift_left(e, 23), f32)


def _make_kernel(TQ, CK, RC, FC, SK, HI, X0, F0, TL):
    NQ = S // TQ
    NC = S // CK
    NR = S // RC
    CPR = RC // CK
    NF = (F - F0) // FC
    assert F0 + NF * FC == F

    def kernel(c_ref, wkt_ref, wvt_ref,
               xt_hbm, wq_hbm, wo_hbm, wmod_hbm, wg_hbm, wu_hbm, wdt_hbm,
               o_ref,
               xt_v, wq_v, wo_v, wmod_v, wg_v, wu_v, wdt_v, sems,
               modt_s, tmp_s, wall_s, wot_s, q_s, mg_s, k_s, ek_s, vt_s, s_s,
               mn_s, ot_s, x1_s, h2_s, acc_s):
        i = pl.program_id(0)

        def cp_mod0():
            return pltpu.make_async_copy(wmod_hbm.at[:, 0:2 * D], wmod_v.at[:, 0:2 * D], sems.at[0])

        def cp_mod1():
            return pltpu.make_async_copy(wmod_hbm.at[:, 2 * D:6 * D], wmod_v.at[:, 2 * D:6 * D], sems.at[1])

        def cp_wg():
            return pltpu.make_async_copy(wg_hbm, wg_v, sems.at[2])

        def cp_wu():
            return pltpu.make_async_copy(wu_hbm, wu_v, sems.at[3])

        def cp_wd():
            return pltpu.make_async_copy(wdt_hbm, wdt_v, sems.at[4])

        def cp_wq():
            return pltpu.make_async_copy(wq_hbm, wq_v, sems.at[5])

        def cp_wo():
            return pltpu.make_async_copy(wo_hbm, wo_v, sems.at[6])

        def cp_x(k):
            sl = slice(0, X0 * RC) if k == 0 else slice(X0 * RC, S)
            return pltpu.make_async_copy(xt_hbm.at[:, sl], xt_v.at[:, sl], sems.at[7 + k])

        def mod_cols(lo, hi):
            cc = c_ref[...].astype(f32)
            sc = cc * (1.0 / (1.0 + jnp.exp(-cc)))
            sc = jnp.broadcast_to(sc, (8, D))
            row = jnp.dot(sc, wmod_v[:, lo:hi], preferred_element_type=f32)[0:1]
            modt_s[lo:hi, :] = jnp.broadcast_to(row, (128, hi - lo)).T

        def col(k, n):
            return jnp.tile(modt_s[k * D:(k + 1) * D, :], (1, n // 128))

        def transpose_w(w_v):
            tmp_s[0:D, 0:D] = w_v[...].astype(f32)
            return tmp_s[...].T[0:D, 0:D]

        def magic(mgq, r):
            return mgq + jnp.tile(ek_s[r], (1, TQ // 128))

        class Head:
            def __init__(self, h, q_off):
                self.q = q_s[h, :, pl.ds(q_off, TQ)]
                self.mgq = mg_s[h, :, pl.ds(q_off, TQ)]
                self.m = None
                self.mb = None

        def a_chunk(hd, c, buf):
            sl = slice(c * CK, (c + 1) * CK)
            if c % CPR == 0:
                hd.mg = magic(hd.mgq, c // CPR)
            n = jnp.dot(k_s[sl, :], hd.q, preferred_element_type=i32)
            s = pltpu.bitcast(n + hd.mg, f32)
            s_s[buf, sl, :] = s
            mc = s.reshape(CK // 8, 8, TQ).max(axis=0)
            hd.mb = mc if hd.mb is None else jnp.maximum(hd.mb, mc)
            if c % CPR == CPR - 1:
                mt = hd.mb - pltpu.bitcast(hd.mg, f32)
                hd.m = mt if hd.m is None else jnp.maximum(hd.m, mt)
                hd.mb = None

        def b_chunk(c, buf, off, acc):
            sl = slice(c * CK, (c + 1) * CK)
            p = jnp.exp2(s_s[buf, sl, :] - off).astype(bf16)
            pv = jnp.dot(vt_s[:, sl], p, preferred_element_type=f32)
            return pv if acc is None else acc + pv

        def b_finish(g, j, acc):
            ot_s[g, j * DH:(j + 1) * DH, :] = (acc * (1.0 / acc[DH:DH + 1]))[0:DH]

        @pl.when(i == 0)
        def _prologue():
            cp_wq().start()
            cp_mod0().start()
            cp_x(0).start()
            cp_x(1).start()
            cp_wo().start()
            cp_mod1().start()

            z6 = jnp.zeros((VR - DH, D), f32)
            wk = jnp.concatenate([wkt_ref[...].astype(f32), z6], axis=0)
            wall_s[0:2 * VR, :] = jnp.concatenate(
                [wvt_ref[...].astype(f32), z6, wk], axis=0).astype(bf16)
            eb = _expo(jnp.broadcast_to(jnp.max(jnp.abs(wk), axis=1, keepdims=True), (VR, 128)))
            kbal = _pow2(254 - eb)
            qbal = _pow2(eb) * QSCALE
            tmp_s[:, D:DP] = jnp.zeros((DP, DP - D), f32)
            tmp_s[D:DP, :] = jnp.zeros((DP - D, DP), f32)

            cp_wq().wait()
            wqt = transpose_w(wq_v)
            for hp in range(H // 2):
                wall_s[2 * VR + 2 * hp * VR:2 * VR + (2 * hp + 2) * VR, :] = jnp.concatenate(
                    [wqt[(2 * hp) * DH:(2 * hp + 1) * DH], z6,
                     wqt[(2 * hp + 1) * DH:(2 * hp + 2) * DH], z6], axis=0).astype(bf16)

            cp_mod0().wait()
            mod_cols(0, 2 * D)

            vrow = lax.broadcasted_iota(i32, (VR, 1), 0)
            clip8 = lambda v: jnp.clip(v, -127.0, 127.0)

            for r in range(NR):
                if r == 0:
                    cp_x(0).wait()
                if r == X0:
                    cp_x(1).wait()
                    cp_wg().start()
                    cp_wu().start()
                    cp_wd().start()
                if r == NR - 1:
                    cp_wo().wait()
                    cp_mod1().wait()
                tok = slice(r * RC, (r + 1) * RC)
                xc = xt_v[:, tok].astype(f32)
                h = (_ln_t(xc) * (1.0 + col(1, RC)) + col(0, RC)).astype(bf16)
                res = jnp.dot(wall_s[...], h, preferred_element_type=f32)
                if r == NR - 1:
                    wot_s[...] = transpose_w(wo_v).astype(bf16)
                vt_s[:, tok] = jnp.where(vrow == DH, 1.0, res[0:VR])

                kt = res[VR:2 * VR] * jnp.tile(kbal, (1, RC // 128))
                kmax = jnp.max(jnp.max(jnp.abs(kt), axis=0, keepdims=True), axis=1, keepdims=True)
                ek = _expo(jnp.broadcast_to(kmax, (1, 128)) * (512.0 / 381.4))
                ek_s[r] = lax.shift_left(ek - 135, 23)
                kt = kt * jnp.tile(_pow2(262 - ek), (1, RC // 128))
                k1 = (kt + RND) - RND
                ka = clip8(k1)
                kb = clip8(k1 - ka)
                kd = jnp.concatenate(
                    [ka, kb, k1 - ka - kb, (kt * (1.0 / T1) + RND) - RND,
                     ((kt - k1) * T2 + RND) - RND, jnp.zeros((8, RC), f32)], axis=0)
                k_s[tok, :] = kd.T.astype(i32).astype(i8)

                qt = res[2 * VR:].reshape(H, VR, RC) * jnp.tile(qbal, (1, RC // 128))[None]
                eq = _expo(jnp.max(jnp.abs(qt), axis=1, keepdims=True) * (128.0 / 127.4))
                mg_s[:, :, tok] = lax.shift_left(eq + 17, 23) + 0x400000
                qt = qt * _pow2(260 - eq)
                t1 = qt + RND
                b1 = pltpu.bitcast(t1, i32)
                ba = pltpu.bitcast((qt - (t1 - RND)) * T1 + RND, i32)
                bc = pltpu.bitcast(qt * (1.0 / T2) + RND, i32)
                qd = jnp.concatenate([b1, b1, b1, ba, bc, jnp.zeros((H, 8, RC), i32)], axis=1)
                q_s[:, :, tok] = qd.astype(i8)

            hd = Head(0, 0)
            for c in range(NC):
                a_chunk(hd, c, 0)
                if c < 9:
                    mod_cols(2 * D + 256 * c, 2 * D + 256 * (c + 1))
            mn_s[...] = hd.m.max(axis=0, keepdims=True)

        q0 = pl.multiple_of(i * TQ, TQ)
        q_next = pl.multiple_of(jnp.minimum(i + 1, NQ - 1) * TQ, TQ)

        b_at = {}
        for jb in range(HI):
            lo = 0 if jb == 0 else jb * NC + SK
            hi = min(lo + NC, HI * NC - TL)
            for cb in range(NC):
                b_at.setdefault(lo + cb * (hi - lo) // NC, []).append((jb, cb))

        def attn_body(it, m_next):
            h0 = it * HI
            g0 = it * (HI // HG)
            last = it == H // HI - 1
            hn = jnp.where(last, 0, h0 + HI)
            qn = pl.multiple_of(jnp.where(last, q_next, q0), TQ)
            ms = {0: m_next}
            mgq = {0: mg_s[h0, :, pl.ds(q0, TQ)]}
            hd = None
            acc = None
            off = None
            for t in range(HI * NC):
                ja, ca = 1 + t // NC, t % NC
                if ca == 0:
                    hd = Head(h0 + ja, q0) if ja < HI else Head(hn, qn)
                    mgq[ja] = hd.mgq
                a_chunk(hd, ca, ja % 2)
                if ca == NC - 1:
                    ms[ja] = hd.m.max(axis=0, keepdims=True)
                for jb, cb in b_at.get(t, ()):
                    if cb % CPR == 0:
                        off = ms[jb] + pltpu.bitcast(magic(mgq[jb], cb // CPR), f32)
                    acc = b_chunk(cb, jb % 2, off, None if cb == 0 else acc)
                    if cb == NC - 1:
                        b_finish(g0 + jb // HG, jb % HG, acc)
            return ms[HI]

        mn_s[...] = lax.fori_loop(0, H // HI, attn_body, mn_s[...])

        @pl.when(i == 0)
        def _():
            cp_wg().wait()
            cp_wu().wait()
            cp_wd().wait()

        def ffn(f0, fc):
            h2 = h2_s[...]
            g = jnp.dot(h2, wg_v[:, pl.ds(f0, fc)], preferred_element_type=f32)
            u = jnp.dot(h2, wu_v[:, pl.ds(f0, fc)], preferred_element_type=f32)
            gh = 0.5 * g
            a = ((gh + gh * jnp.tanh(gh)) * u).astype(bf16)
            return lax.dot_general(wdt_v[:, pl.ds(f0, fc)], a, NT, preferred_element_type=f32)

        ot = ot_s[...].reshape(D, TQ).astype(bf16)
        attn = jnp.dot(wot_s[...], ot, preferred_element_type=f32)
        x1 = xt_v[:, pl.ds(q0, TQ)].astype(f32) + col(2, TQ) * attn
        x1_s[...] = x1
        h2t = _ln_t(x1) * (1.0 + col(4, TQ)) + col(3, TQ)
        h2t = jnp.concatenate([h2t, jnp.zeros((DP - D, TQ), f32)], axis=0)
        h2_s[...] = h2t.T[:, 0:D].astype(bf16)
        acc_s[...] = ffn(0, F0)

        def ffn_body(fi, carry):
            f0 = pl.multiple_of(F0 + fi * FC, 128)
            y = acc_s[...] + ffn(f0, FC)
            acc_s[...] = y
            o_ref[...] = (x1_s[...] + col(5, TQ) * y).astype(o_ref.dtype)
            return carry

        lax.fori_loop(0, NF, ffn_body, 0)

    return kernel


@functools.partial(jax.jit, static_argnames=("TQ", "CK", "RC", "FC", "SK", "HI", "X0", "F0", "TL"))
def _run(A_x, A_wq, A_wk, A_wv, A_wo, B_x, B_w_gate, B_w_up, B_w_down, c, w_mod,
        TQ=512, CK=128, RC=512, FC=1280, SK=2, HI=8, X0=1, F0=768, TL=1):
    xt = A_x.reshape(S, D).T
    full = lambda shape: pl.BlockSpec(shape, lambda i: (0,) * len(shape))
    hbm = pl.BlockSpec(memory_space=pltpu.HBM)
    out = pl.pallas_call(
        _make_kernel(TQ, CK, RC, FC, SK, HI, X0, F0, TL),
        grid=(S // TQ,),
        in_specs=[full((1, D)), full((DH, D)), full((DH, D))] + [hbm] * 7,
        out_specs=pl.BlockSpec((D, TQ), lambda i: (0, i)),
        out_shape=jax.ShapeDtypeStruct((D, S), bf16),
        scratch_shapes=[
            pltpu.VMEM((D, S), bf16),
            pltpu.VMEM((D, D), bf16),
            pltpu.VMEM((D, D), bf16),
            pltpu.VMEM((D, 6 * D), bf16),
            pltpu.VMEM((D, F), bf16),
            pltpu.VMEM((D, F), bf16),
            pltpu.VMEM((D, F), bf16),
            pltpu.SemaphoreType.DMA((9,)),
            pltpu.VMEM((6 * D, 128), f32),
            pltpu.VMEM((DP, DP), f32),
            pltpu.VMEM(((H + 2) * VR, D), bf16),
            pltpu.VMEM((D, D), bf16),
            pltpu.VMEM((H, 128, S), i8),
            pltpu.VMEM((H, 1, S), i32),
            pltpu.VMEM((S, 128), i8),
            pltpu.VMEM((S // RC, 1, 128), i32),
            pltpu.VMEM((VR, S), f32),
            pltpu.VMEM((2, S, TQ), f32),
            pltpu.VMEM((1, TQ), f32),
            pltpu.VMEM((NG, HG * DH, TQ), f32),
            pltpu.VMEM((D, TQ), f32),
            pltpu.VMEM((TQ, D), bf16),
            pltpu.VMEM((D, TQ), f32),
        ],
        compiler_params=pltpu.CompilerParams(
            dimension_semantics=("arbitrary",),
            vmem_limit_bytes=100 * 1024 * 1024),
    )(c, A_wk.T, A_wv.T, xt, A_wq, A_wo, w_mod, B_w_gate, B_w_up, B_w_down.T)
    return out.T.reshape(1, S, D)


@jax.jit
def pallas_adaLN_cond__grouped_kv_mqa__swiglu_ffn__prompt_kernel(
    A_x: jax.Array,
    A_wq: jax.Array,
    A_wk: jax.Array,
    A_wv: jax.Array,
    A_wo: jax.Array,
    B_x: jax.Array,
    B_w_gate: jax.Array,
    B_w_up: jax.Array,
    B_w_down: jax.Array,
    c: jax.Array,
    w_mod: jax.Array,
):
    return _run(A_x, A_wq, A_wk, A_wv, A_wo, B_x, B_w_gate, B_w_up, B_w_down, c, w_mod)
```

```python
import math

import jax
import jax.numpy as jnp
from jax import lax
import jax.experimental.pallas as pl
import jax.experimental.pallas.tpu as pltpu

f32 = jnp.float32
bf16 = jnp.bfloat16
i32 = jnp.int32
i8 = jnp.int8

S = 2048
D = 576
H = 32
DH = 18
F = 4608
DP = 640
HG = 4
NG = H // HG
VR = 24
EPS = 1e-5
QSCALE = DH ** -0.5 * math.log2(math.e)
NT = (((1,), (1,)), ((), ()))
RND = 1.5 * 2.0 ** 23
T1 = 16.0
T2 = 16.0

TQ = 512
CK = 128
HI = 8
G = 3
SK = 9
TL = 3
F0 = 768
FC = 1280

NQ = S // TQ
NC = S // CK
CPR = TQ // CK
QT = TQ // 128
NTL = NC * QT
TOT = HI * NTL
NF = (F - F0) // FC
assert F0 + NF * FC == F


def _ln_t(x):
    mu = jnp.mean(x, axis=0, keepdims=True)
    xc = x - mu
    var = jnp.mean(xc * xc, axis=0, keepdims=True)
    return xc * lax.rsqrt(var + EPS)


def _expo(a, lo, hi):
    a = jnp.minimum(jnp.maximum(a, 2.0 ** lo), 2.0 ** hi)
    return pltpu.bitcast(a, i32) & 0x7F800000


def _pow2(bits):
    return pltpu.bitcast(bits, f32)


def _inv2(bits):
    return pltpu.bitcast((254 << 23) - bits, f32)


def _lanes(v, k):
    return v[:, k * 128:(k + 1) * 128]


def _runs(n0, n1):
    out = []
    while n0 < n1:
        hd, r = divmod(n0, NTL)
        c, qt = divmod(r, QT)
        e = min(QT, qt + n1 - n0)
        out.append((hd, c, qt, e))
        n0 += e - qt
    return out


def _b_target(a_done):
    best = 0
    for jb in range(HI):
        lo = 0 if jb == 0 else jb * NTL + SK
        hi = min(lo + NTL, TOT - TL)
        if a_done > lo:
            best = jb * NTL + min(NTL, -(-(a_done - lo) * NTL // (hi - lo)))
    return best


def _kernel(c_hbm, wkt_hbm, wvt_hbm, xt_hbm, wq_hbm, wo_hbm, wmod_hbm, wg_hbm, wu_hbm, wdt_hbm,
            o_ref,
            xt_v, wq_v, wo_v, wmod_v, wg_v, wu_v, wdt_v, sems,
            modt_s, tmp_s, wot_s, q_s, mg_s, k_s, ek_s, vt_s, s_s,
            mn_s, ot_s, x1_s, h2_s, acc_s, wall_s, wkt_v, wvt_v, c_v):
    i = pl.program_id(0)

    def cp_cols(src, dst, lo, hi, k):
        return pltpu.make_async_copy(src.at[:, lo:hi], dst.at[:, lo:hi], sems.at[k])

    cp_mod0 = lambda: cp_cols(wmod_hbm, wmod_v, 0, 2 * D, 0)
    cp_mod1 = lambda: cp_cols(wmod_hbm, wmod_v, 2 * D, 6 * D, 1)
    cp_x0 = lambda: cp_cols(xt_hbm, xt_v, 0, TQ, 2)
    cp_x1 = lambda: cp_cols(xt_hbm, xt_v, TQ, S, 3)
    cp_wo = lambda: pltpu.make_async_copy(wo_hbm, wo_v, sems.at[4])
    cp_first = lambda: [
        pltpu.make_async_copy(src, dst, sems.at[5 + k]) for k, (src, dst) in enumerate(
            ((wq_hbm, wq_v), (wkt_hbm, wkt_v), (wvt_hbm, wvt_v), (c_hbm, c_v)))]
    cp_ffn = lambda: [
        pltpu.make_async_copy(src, dst, sems.at[9 + k]) for k, (src, dst) in enumerate(
            ((wg_hbm, wg_v), (wu_hbm, wu_v), (wdt_hbm, wdt_v)))]

    def mod_cols(lo, hi):
        cc = c_v[...].astype(f32)
        sc = jnp.broadcast_to(cc * (1.0 / (1.0 + jnp.exp(-cc))), (8, D))
        row = jnp.dot(sc, wmod_v[:, lo:hi], preferred_element_type=f32)[0:1]
        lane = lax.broadcasted_iota(i32, (1, hi - lo), 1) + lo
        scale = ((lane >= D) & (lane < 2 * D)) | ((lane >= 4 * D) & (lane < 5 * D))
        row = jnp.where(scale, row + 1.0, row)
        modt_s[lo:hi, :] = jnp.broadcast_to(row, (128, hi - lo)).T

    def col(k):
        return jnp.tile(modt_s[k * D:(k + 1) * D, :], (1, QT))

    def transpose_w(w_v):
        tmp_s[0:D, 0:D] = w_v[...].astype(f32)
        return tmp_s[...].T[0:D, 0:D]

    class Head:
        def __init__(self, h, m=None):
            self.h = h
            self.mgq = mg_s[h]
            self.mg = {}
            self.mb = {}
            self.mt = {}
            self.m = m
            self.off = {}
            self.acc = {}

        def bias_bits(self, qt, r):
            return _lanes(self.mgq, qt) + ek_s[r]

    def a_run(hd, j, c, q0t, q1t, buf):
        if c % CPR == 0:
            for qt in range(q0t, q1t):
                hd.mg[qt] = hd.bias_bits(qt, c // CPR)
        mg = jnp.concatenate([hd.mg[qt] for qt in range(q0t, q1t)], axis=1)
        qd = pltpu.bitcast(q_s[hd.h, :, q0t * 128:q1t * 128], i8)
        kd = pltpu.bitcast(k_s[j, c * (CK // 4):(c + 1) * (CK // 4), :], i8)
        n = jnp.dot(kd, qd, preferred_element_type=i32)
        s = pltpu.bitcast(n + jnp.tile(mg, (CK // 8, 1)), f32)
        s_s[buf, c * CK:(c + 1) * CK, q0t * 128:q1t * 128] = s
        mc = s.reshape(CK // 8, 8, (q1t - q0t) * 128).max(axis=0)
        for qt in range(q0t, q1t):
            v = _lanes(mc, qt - q0t)
            hd.mb[qt] = v if c % CPR == 0 else jnp.maximum(hd.mb[qt], v)
            if c % CPR == CPR - 1:
                v = hd.mb[qt] - pltpu.bitcast(hd.mg[qt], f32)
                hd.mt[qt] = v if c < CPR else jnp.maximum(hd.mt[qt], v)
        if c == NC - 1 and q1t == QT:
            m = jnp.concatenate([hd.mt[qt] for qt in range(QT)], axis=1)
            hd.m = jnp.broadcast_to(m.max(axis=0, keepdims=True), (8, TQ))

    def b_run(hd, c, q0t, q1t, buf, g, j):
        sl = slice(c * CK, (c + 1) * CK)
        if c % CPR == 0:
            for qt in range(q0t, q1t):
                hd.off[qt] = _lanes(hd.m, qt) + pltpu.bitcast(hd.bias_bits(qt, c // CPR), f32)
        off = jnp.concatenate([hd.off[qt] for qt in range(q0t, q1t)], axis=1)
        p = jnp.exp2(s_s[buf, sl, q0t * 128:q1t * 128] - jnp.tile(off, (CK // 8, 1)))
        pv = jnp.dot(vt_s[:, sl], p.astype(bf16), preferred_element_type=f32)
        for qt in range(q0t, q1t):
            v = _lanes(pv, qt - q0t)
            acc = hd.acc[qt] = v if c == 0 else hd.acc[qt] + v
            if c == NC - 1:
                ot_s[g, j * DH:(j + 1) * DH, qt * 128:(qt + 1) * 128] = (
                    acc * (1.0 / acc[DH:DH + 1]))[0:DH]

    @pl.when(i == 0)
    def _prologue():
        for cp in cp_first():
            cp.start()
        cp_mod0().start()
        cp_x0().start()
        cp_x1().start()
        cp_wo().start()
        cp_mod1().start()

        tmp_s[:, D:DP] = jnp.zeros((DP, DP - D), f32)
        tmp_s[D:DP, :] = jnp.zeros((DP - D, DP), f32)

        for cp in cp_first():
            cp.wait()
        z6 = jnp.zeros((VR - DH, D), f32)
        wk = jnp.concatenate([wkt_v[...].astype(f32), z6], axis=0)
        wall_s[0:2 * VR, :] = jnp.concatenate([wvt_v[...].astype(f32), z6, wk], axis=0).astype(bf16)
        eb = _expo(jnp.broadcast_to(jnp.max(jnp.abs(wk), axis=1, keepdims=True), (VR, 128)),
                   -60, 60)
        kbal = _inv2(eb) * QSCALE
        qbal = jnp.concatenate([_pow2(eb)[0:DH]] * HG, axis=0)
        qbal = jnp.tile(qbal, (NG, DP // 128))[:, 0:D]
        wall_s[2 * VR:, :] = (transpose_w(wq_v) * qbal).astype(bf16)

        cp_mod0().wait()
        mod_cols(0, 2 * D)

        vrow = lax.broadcasted_iota(i32, (VR, 1), 0)
        row8 = lax.broadcasted_iota(i32, (1, 8, 1), 1)
        clip8 = lambda v: jnp.clip(v, -127.0, 127.0)

        for r in range(NQ):
            if r == 0:
                cp_x0().wait()
            if r == 1:
                cp_x1().wait()
                for cp in cp_ffn():
                    cp.start()
            if r == NQ - 1:
                cp_wo().wait()
                cp_mod1().wait()
            tok = slice(r * TQ, (r + 1) * TQ)
            h = (_ln_t(xt_v[:, tok].astype(f32)) * col(1) + col(0)).astype(bf16)
            res = jnp.dot(wall_s[...], h, preferred_element_type=f32)
            if r == NQ - 1:
                wot_s[...] = transpose_w(wo_v).astype(bf16)
            vt_s[:, tok] = jnp.where(vrow == DH, 1.0, res[0:VR])

            kt = res[VR:2 * VR] * jnp.tile(kbal, (1, QT))
            kmax = jnp.max(jnp.max(jnp.abs(kt), axis=0, keepdims=True), axis=1, keepdims=True)
            ek = _expo(jnp.broadcast_to(kmax, (8, 128)) * (512.0 / 381.4), -30, 30)
            ek_s[r] = ek - (135 << 23)
            kt = kt * jnp.tile(_inv2(ek) * 256.0, (VR // 8, QT))
            k1 = (kt + RND) - RND
            ka = clip8(k1)
            kb = clip8(k1 - ka)
            kd = jnp.concatenate(
                [ka + RND, kb + RND, (k1 - ka - kb) + RND, kt * (1.0 / T1) + RND,
                 (kt - k1) * T2 + RND, jnp.zeros((8, TQ), f32)], axis=0)
            kd = pltpu.bitcast(pltpu.bitcast(kd.T, i32).astype(i8), i32)
            for j in range(HG):
                k_s[j, r * (TQ // 4):(r + 1) * (TQ // 4), :] = (
                    kd if j == 0 else pltpu.roll(kd, 2 * j, 1))

            qt = res[2 * VR:].reshape(NG, HG * DH, TQ)
            qa = jnp.abs(qt)
            inv = []
            for j in range(HG):
                w = [qa[:, 16 * j + 8 * t:16 * j + 8 * (t + 1)] for t in range(3)]
                if j > 0:
                    w[0] = jnp.where(row8 >= 2 * j, w[0], 0.0)
                if j < HG - 1:
                    w[2] = jnp.where(row8 < 2 * j + 2, w[2], 0.0)
                amax = jnp.max(jnp.maximum(jnp.maximum(w[0], w[1]), w[2]), axis=1, keepdims=True)
                eq = jnp.broadcast_to(_expo(amax * (2.0 / 127.4), -106, 80), (NG, 8, TQ))
                for g in range(NG):
                    mg_s[r * H + g * HG + j] = eq[g] + ((23 << 23) + 0x400000)
                inv.append(_inv2(eq))
            mix = lambda j: jnp.where(row8 < 2 * j + 2, inv[j], inv[j + 1])
            qt = qt * jnp.concatenate(
                [inv[0], inv[0], mix(0), inv[1], mix(1), inv[2], mix(2), inv[3], inv[3]], axis=1)
            t1 = qt + RND
            b1 = pltpu.bitcast(t1, i32)
            ba = pltpu.bitcast((qt - (t1 - RND)) * T1 + RND, i32)
            bc = pltpu.bitcast(qt * (1.0 / T2) + RND, i32)
            for j in range(HG):
                win = slice(16 * j, 16 * j + VR)
                qd = jnp.concatenate(
                    [b1[:, win], b1[:, win], b1[:, win], ba[:, win], bc[:, win],
                     jnp.zeros((NG, 8, TQ), i32)], axis=1)
                qd = pltpu.bitcast(qd.astype(i8), i32)
                for g in range(NG):
                    q_s[r * H + g * HG + j] = qd[g]

        hd = Head(0)
        for c in range(NC):
            a_run(hd, 0, c, 0, QT, 0)
            if c < 9:
                mod_cols(2 * D + 256 * c, 2 * D + 256 * (c + 1))
        mn_s[...] = hd.m

    def attn_body(it, m_next):
        h0 = i * H + it * HI
        g0 = it * (HI // HG)
        hn = jnp.minimum(h0 + HI, NQ * H - HG)
        heads = {0: Head(h0, m_next)}
        a_done = b_done = 0
        while a_done < TOT:
            a1 = min(TOT, a_done + G)
            for ha, c, q0t, q1t in _runs(a_done, a1):
                ja = ha + 1
                if ja not in heads:
                    heads[ja] = Head(h0 + ja if ja < HI else hn)
                a_run(heads[ja], ja % HG, c, q0t, q1t, ja % 2)
            a_done = a1
            b1 = _b_target(a_done)
            for jb, c, q0t, q1t in _runs(b_done, b1):
                b_run(heads[jb], c, q0t, q1t, jb % 2, g0 + jb // HG, jb % HG)
            b_done = b1
        assert b_done == TOT
        return heads[HI].m

    mn_s[...] = lax.fori_loop(0, H // HI, attn_body, mn_s[...])

    @pl.when(i == 0)
    def _():
        for cp in cp_ffn():
            cp.wait()

    def ffn(f0, fc):
        h2 = h2_s[...]
        g = jnp.dot(h2, wg_v[:, pl.ds(f0, fc)], preferred_element_type=f32)
        u = jnp.dot(h2, wu_v[:, pl.ds(f0, fc)], preferred_element_type=f32)
        gh = 0.5 * g
        a = ((gh + gh * jnp.tanh(gh)) * u).astype(bf16)
        return lax.dot_general(wdt_v[:, pl.ds(f0, fc)], a, NT, preferred_element_type=f32)

    q0 = pl.multiple_of(i * TQ, TQ)
    ot = ot_s[...].reshape(D, TQ).astype(bf16)
    attn = jnp.dot(wot_s[...], ot, preferred_element_type=f32)
    x1 = xt_v[:, pl.ds(q0, TQ)].astype(f32) + col(2) * attn
    x1_s[...] = x1
    h2t = _ln_t(x1) * col(4) + col(3)
    h2t = jnp.concatenate([h2t, jnp.zeros((DP - D, TQ), f32)], axis=0)
    h2_s[...] = h2t.T[:, 0:D].astype(bf16)
    acc_s[...] = ffn(0, F0)

    def ffn_body(fi, carry):
        f0 = pl.multiple_of(F0 + fi * FC, 128)
        y = acc_s[...] + ffn(f0, FC)
        acc_s[...] = y
        o_ref[...] = (x1_s[...] + col(5) * y).astype(o_ref.dtype)
        return carry

    lax.fori_loop(0, NF, ffn_body, 0)


@jax.jit
def pallas_adaLN_cond__grouped_kv_mqa__swiglu_ffn__prompt_kernel(
    A_x: jax.Array,
    A_wq: jax.Array,
    A_wk: jax.Array,
    A_wv: jax.Array,
    A_wo: jax.Array,
    B_x: jax.Array,
    B_w_gate: jax.Array,
    B_w_up: jax.Array,
    B_w_down: jax.Array,
    c: jax.Array,
    w_mod: jax.Array,
):
    del B_x
    out_t = pl.pallas_call(
        _kernel,
        grid=(NQ,),
        in_specs=[pl.BlockSpec(memory_space=pltpu.HBM)] * 10,
        out_specs=pl.BlockSpec((D, TQ), lambda i: (0, i)),
        out_shape=jax.ShapeDtypeStruct((D, S), bf16),
        scratch_shapes=[
            pltpu.VMEM((D, S), bf16),
            pltpu.VMEM((D, D), bf16),
            pltpu.VMEM((D, D), bf16),
            pltpu.VMEM((D, 6 * D), bf16),
            pltpu.VMEM((D, F), bf16),
            pltpu.VMEM((D, F), bf16),
            pltpu.VMEM((D, F), bf16),
            pltpu.SemaphoreType.DMA((12,)),
            pltpu.VMEM((6 * D, 128), f32),
            pltpu.VMEM((DP, DP), f32),
            pltpu.VMEM((D, D), bf16),
            pltpu.VMEM((NQ * H, 32, TQ), i32),
            pltpu.VMEM((NQ * H, 8, TQ), i32),
            pltpu.VMEM((HG, S // 4, 128), i32),
            pltpu.VMEM((NQ, 8, 128), i32),
            pltpu.VMEM((VR, S), f32),
            pltpu.VMEM((2, S, TQ), f32),
            pltpu.VMEM((8, TQ), f32),
            pltpu.VMEM((NG, HG * DH, TQ), f32),
            pltpu.VMEM((D, TQ), f32),
            pltpu.VMEM((TQ, D), bf16),
            pltpu.VMEM((D, TQ), f32),
            pltpu.VMEM((2 * VR + D, D), bf16),
            pltpu.VMEM((DH, D), bf16),
            pltpu.VMEM((DH, D), bf16),
            pltpu.VMEM((1, D), bf16),
        ],
        compiler_params=pltpu.CompilerParams(
            dimension_semantics=("arbitrary",),
            vmem_limit_bytes=100 * 1024 * 1024),
    )(c, A_wk.T, A_wv.T, A_x.reshape(S, D).T, A_wq, A_wo, w_mod, B_w_gate, B_w_up, B_w_down.T)
    return out_t.T.reshape(1, S, D)
```

```python
import math

import jax
import jax.numpy as jnp
from jax import lax
import jax.experimental.pallas as pl
import jax.experimental.pallas.tpu as pltpu

f32 = jnp.float32
bf16 = jnp.bfloat16
i32 = jnp.int32
i8 = jnp.int8

S = 2048
D = 576
H = 32
DH = 18
F = 4608
DP = 640
HG = 4
NG = H // HG
VR = 24
EPS = 1e-5
QSCALE = DH ** -0.5 * math.log2(math.e)
NT = (((1,), (1,)), ((), ()))
RND = 1.5 * 2.0 ** 23
T1 = 16.0
T2 = 16.0

TQ = 512
CK = 128
HI = 8
G = 3
SK = 9
TL = 3
F0 = 768
FC = 1280

NQ = S // TQ
NC = S // CK
CPR = TQ // CK
QT = TQ // 128
NTL = NC * QT
TOT = HI * NTL
NF = (F - F0) // FC
assert F0 + NF * FC == F


def _ln_t(x):
    def mean0(v):
        v = v.reshape(D // 16, 16, v.shape[1]).sum(axis=0)
        return jnp.sum(v, axis=0, keepdims=True) * (1.0 / D)

    xc = x - mean0(x)
    return xc * lax.rsqrt(mean0(xc * xc) + EPS)


def _expo(a, lo, hi):
    a = jnp.minimum(jnp.maximum(a, 2.0 ** lo), 2.0 ** hi)
    return pltpu.bitcast(a, i32) & 0x7F800000


def _pow2(bits):
    return pltpu.bitcast(bits, f32)


def _inv2(bits):
    return pltpu.bitcast((254 << 23) - bits, f32)


def _lanes(v, k):
    return v[:, k * 128:(k + 1) * 128]


def _runs(n0, n1):
    out = []
    while n0 < n1:
        hd, r = divmod(n0, NTL)
        c, qt = divmod(r, QT)
        e = min(QT, qt + n1 - n0)
        out.append((hd, c, qt, e))
        n0 += e - qt
    return out


def _b_target(a_done):
    best = 0
    for jb in range(HI):
        lo = 0 if jb == 0 else jb * NTL + SK
        hi = min(lo + NTL, TOT - TL)
        if a_done > lo:
            best = jb * NTL + min(NTL, -(-(a_done - lo) * NTL // (hi - lo)))
    return best


def _kernel(c_hbm, wkt_hbm, wvt_hbm, xt_hbm, wq_hbm, wo_hbm, wmod_hbm, wg_hbm, wu_hbm, wdt_hbm,
            o_ref,
            xt_v, wq_v, wo_v, wmod_v, wg_v, wu_v, wdt_v, sems,
            modt_s, tmp_s, wot_s, q_s, mg_s, k_s, ek_s, vt_s, s_s,
            mn_s, ot_s, x1_s, h2_s, acc_s, wall_s, wkt_v, wvt_v, c_v):
    i = pl.program_id(0)

    def cp_cols(src, dst, lo, hi, k):
        return pltpu.make_async_copy(src.at[:, lo:hi], dst.at[:, lo:hi], sems.at[k])

    cp_mod0 = lambda: cp_cols(wmod_hbm, wmod_v, 0, 2 * D, 0)
    cp_mod1 = lambda: cp_cols(wmod_hbm, wmod_v, 2 * D, 6 * D, 1)
    cp_x0 = lambda: cp_cols(xt_hbm, xt_v, 0, TQ, 2)
    cp_x1 = lambda: cp_cols(xt_hbm, xt_v, TQ, S, 3)
    cp_wo = lambda: pltpu.make_async_copy(wo_hbm, wo_v, sems.at[4])
    cp_first = lambda: [
        pltpu.make_async_copy(src, dst, sems.at[5 + k]) for k, (src, dst) in enumerate(
            ((wq_hbm, wq_v), (wkt_hbm, wkt_v), (wvt_hbm, wvt_v), (c_hbm, c_v)))]
    cp_ffn = lambda: [
        pltpu.make_async_copy(src, dst, sems.at[9 + k]) for k, (src, dst) in enumerate(
            ((wg_hbm, wg_v), (wu_hbm, wu_v), (wdt_hbm, wdt_v)))]

    def mod_cols(lo, hi):
        cc = c_v[...].astype(f32)
        sc = jnp.broadcast_to(cc * (1.0 / (1.0 + jnp.exp(-cc))), (8, D))
        row = jnp.dot(sc, wmod_v[:, lo:hi], preferred_element_type=f32)[0:1]
        lane = lax.broadcasted_iota(i32, (1, hi - lo), 1) + lo
        scale = ((lane >= D) & (lane < 2 * D)) | ((lane >= 4 * D) & (lane < 5 * D))
        row = jnp.where(scale, row + 1.0, row)
        modt_s[lo:hi, :] = jnp.broadcast_to(row, (128, hi - lo)).T

    def col(k):
        return jnp.tile(modt_s[k * D:(k + 1) * D, :], (1, QT))

    def transpose_w(w_v):
        tmp_s[0:D, 0:D] = w_v[...].astype(f32)
        return tmp_s[...].T[0:D, 0:D]

    class Head:
        def __init__(self, h, m=None):
            self.h = h
            self.mgq = mg_s[h]
            self.mg = {}
            self.mb = {}
            self.mt = {}
            self.m = m
            self.off = {}
            self.acc = {}

        def bias_bits(self, qt, r):
            return _lanes(self.mgq, qt) + ek_s[r]

    def a_run(hd, j, c, q0t, q1t, buf):
        if c % CPR == 0:
            for qt in range(q0t, q1t):
                hd.mg[qt] = hd.bias_bits(qt, c // CPR)
        mg = jnp.concatenate([hd.mg[qt] for qt in range(q0t, q1t)], axis=1)
        qd = pltpu.bitcast(q_s[hd.h, :, q0t * 128:q1t * 128], i8)
        kd = pltpu.bitcast(k_s[j, c * (CK // 4):(c + 1) * (CK // 4), :], i8)
        n = jnp.dot(kd, qd, preferred_element_type=i32)
        s = pltpu.bitcast(n + jnp.tile(mg, (CK // 8, 1)), f32)
        s_s[buf, c * CK:(c + 1) * CK, q0t * 128:q1t * 128] = s
        mc = s.reshape(CK // 8, 8, (q1t - q0t) * 128).max(axis=0)
        for qt in range(q0t, q1t):
            v = _lanes(mc, qt - q0t)
            hd.mb[qt] = v if c % CPR == 0 else jnp.maximum(hd.mb[qt], v)
            if c % CPR == CPR - 1:
                v = hd.mb[qt] - pltpu.bitcast(hd.mg[qt], f32)
                hd.mt[qt] = v if c < CPR else jnp.maximum(hd.mt[qt], v)
        if c == NC - 1 and q1t == QT:
            m = jnp.concatenate([hd.mt[qt] for qt in range(QT)], axis=1)
            hd.m = jnp.broadcast_to(m.max(axis=0, keepdims=True), (8, TQ))

    def b_run(hd, c, q0t, q1t, buf, g, j):
        sl = slice(c * CK, (c + 1) * CK)
        if c % CPR == 0:
            for qt in range(q0t, q1t):
                hd.off[qt] = _lanes(hd.m, qt) + pltpu.bitcast(hd.bias_bits(qt, c // CPR), f32)
        off = jnp.concatenate([hd.off[qt] for qt in range(q0t, q1t)], axis=1)
        p = jnp.exp2(s_s[buf, sl, q0t * 128:q1t * 128] - jnp.tile(off, (CK // 8, 1)))
        pv = jnp.dot(vt_s[:, sl], p.astype(bf16), preferred_element_type=f32)
        for qt in range(q0t, q1t):
            v = _lanes(pv, qt - q0t)
            acc = hd.acc[qt] = v if c == 0 else hd.acc[qt] + v
            if c == NC - 1:
                ot_s[g, j * DH:(j + 1) * DH, qt * 128:(qt + 1) * 128] = (
                    acc * (1.0 / acc[DH:DH + 1]))[0:DH]

    @pl.when(i == 0)
    def _prologue():
        for cp in cp_first():
            cp.start()
        cp_mod0().start()
        cp_x0().start()
        cp_x1().start()
        cp_wo().start()
        cp_mod1().start()

        tmp_s[:, D:DP] = jnp.zeros((DP, DP - D), f32)
        tmp_s[D:DP, :] = jnp.zeros((DP - D, DP), f32)

        for cp in cp_first():
            cp.wait()
        z6 = jnp.zeros((VR - DH, D), f32)
        wk = jnp.concatenate([wkt_v[...].astype(f32), z6], axis=0)
        wall_s[0:2 * VR, :] = jnp.concatenate([wvt_v[...].astype(f32), z6, wk], axis=0).astype(bf16)
        eb = _expo(jnp.broadcast_to(jnp.max(jnp.abs(wk), axis=1, keepdims=True), (VR, 128)),
                   -60, 60)
        kbal = _inv2(eb) * QSCALE
        qbal = jnp.concatenate([_pow2(eb)[0:DH]] * HG, axis=0)
        qbal = jnp.tile(qbal, (NG, DP // 128))[:, 0:D]
        wall_s[2 * VR:, :] = (transpose_w(wq_v) * qbal).astype(bf16)

        cp_mod0().wait()
        mod_cols(0, 2 * D)

        vrow = lax.broadcasted_iota(i32, (VR, 1), 0)
        row8 = lax.broadcasted_iota(i32, (1, 8, 1), 1)
        clip8 = lambda v: jnp.clip(v, -127.0, 127.0)

        for r in range(NQ):
            if r == 0:
                cp_x0().wait()
            if r == 1:
                cp_x1().wait()
                for cp in cp_ffn():
                    cp.start()
            if r == NQ - 1:
                cp_wo().wait()
                cp_mod1().wait()
            tok = slice(r * TQ, (r + 1) * TQ)
            h = (_ln_t(xt_v[:, tok].astype(f32)) * col(1) + col(0)).astype(bf16)
            res = jnp.dot(wall_s[...], h, preferred_element_type=f32)
            if r == NQ - 1:
                wot_s[...] = transpose_w(wo_v).astype(bf16)
            vt_s[:, tok] = jnp.where(vrow == DH, 1.0, res[0:VR])

            kt = res[VR:2 * VR] * jnp.tile(kbal, (1, QT))
            kmax = jnp.max(jnp.max(jnp.abs(kt), axis=0, keepdims=True), axis=1, keepdims=True)
            ek = _expo(jnp.broadcast_to(kmax, (8, 128)) * (512.0 / 381.4), -30, 30)
            ek_s[r] = ek - (135 << 23)
            kt = kt * jnp.tile(_inv2(ek) * 256.0, (VR // 8, QT))
            k1 = (kt + RND) - RND
            ka = clip8(k1)
            kb = clip8(k1 - ka)
            kd = jnp.concatenate(
                [ka + RND, kb + RND, (k1 - ka - kb) + RND, kt * (1.0 / T1) + RND,
                 (kt - k1) * T2 + RND, jnp.zeros((8, TQ), f32)], axis=0)
            kd = pltpu.bitcast(pltpu.bitcast(kd.T, i32).astype(i8), i32)
            for j in range(HG):
                k_s[j, r * (TQ // 4):(r + 1) * (TQ // 4), :] = (
                    kd if j == 0 else pltpu.roll(kd, 2 * j, 1))

            qt = res[2 * VR:].reshape(NG, HG * DH, TQ)
            qa = jnp.abs(qt)
            inv = []
            for j in range(HG):
                w = [qa[:, 16 * j + 8 * t:16 * j + 8 * (t + 1)] for t in range(3)]
                if j > 0:
                    w[0] = jnp.where(row8 >= 2 * j, w[0], 0.0)
                if j < HG - 1:
                    w[2] = jnp.where(row8 < 2 * j + 2, w[2], 0.0)
                amax = jnp.max(jnp.maximum(jnp.maximum(w[0], w[1]), w[2]), axis=1, keepdims=True)
                eq = jnp.broadcast_to(_expo(amax * (2.0 / 127.4), -106, 80), (NG, 8, TQ))
                for g in range(NG):
                    mg_s[r * H + g * HG + j] = eq[g] + ((23 << 23) + 0x400000)
                inv.append(_inv2(eq))
            mix = lambda j: jnp.where(row8 < 2 * j + 2, inv[j], inv[j + 1])
            qt = qt * jnp.concatenate(
                [inv[0], inv[0], mix(0), inv[1], mix(1), inv[2], mix(2), inv[3], inv[3]], axis=1)
            t1 = qt + RND
            b1 = pltpu.bitcast(t1, i32)
            ba = pltpu.bitcast((qt - (t1 - RND)) * T1 + RND, i32)
            bc = pltpu.bitcast(qt * (1.0 / T2) + RND, i32)
            for j in range(HG):
                win = slice(16 * j, 16 * j + VR)
                qd = jnp.concatenate(
                    [b1[:, win], b1[:, win], b1[:, win], ba[:, win], bc[:, win],
                     jnp.zeros((NG, 8, TQ), i32)], axis=1)
                qd = pltpu.bitcast(qd.astype(i8), i32)
                for g in range(NG):
                    q_s[r * H + g * HG + j] = qd[g]

        hd = Head(0)
        for c in range(NC):
            a_run(hd, 0, c, 0, QT, 0)
            if c < 9:
                mod_cols(2 * D + 256 * c, 2 * D + 256 * (c + 1))
        mn_s[...] = hd.m

    def attn_body(it, m_next):
        h0 = i * H + it * HI
        g0 = it * (HI // HG)
        hn = jnp.minimum(h0 + HI, NQ * H - HG)
        heads = {0: Head(h0, m_next)}
        a_done = b_done = 0
        while a_done < TOT:
            a1 = min(TOT, a_done + G)
            for ha, c, q0t, q1t in _runs(a_done, a1):
                ja = ha + 1
                if ja not in heads:
                    heads[ja] = Head(h0 + ja if ja < HI else hn)
                a_run(heads[ja], ja % HG, c, q0t, q1t, ja % 2)
            a_done = a1
            b1 = _b_target(a_done)
            for jb, c, q0t, q1t in _runs(b_done, b1):
                b_run(heads[jb], c, q0t, q1t, jb % 2, g0 + jb // HG, jb % HG)
            b_done = b1
        assert b_done == TOT
        return heads[HI].m

    mn_s[...] = lax.fori_loop(0, H // HI, attn_body, mn_s[...])

    @pl.when(i == 0)
    def _():
        for cp in cp_ffn():
            cp.wait()

    def ffn(f0, fc):
        h2 = h2_s[...]
        g = jnp.dot(h2, wg_v[:, pl.ds(f0, fc)], preferred_element_type=f32)
        u = jnp.dot(h2, wu_v[:, pl.ds(f0, fc)], preferred_element_type=f32)
        gh = 0.5 * g
        a = ((gh + gh * jnp.tanh(gh)) * u).astype(bf16)
        return lax.dot_general(wdt_v[:, pl.ds(f0, fc)], a, NT, preferred_element_type=f32)

    q0 = pl.multiple_of(i * TQ, TQ)
    ot = ot_s[...].reshape(D, TQ).astype(bf16)
    attn = jnp.dot(wot_s[...], ot, preferred_element_type=f32)
    x1 = xt_v[:, pl.ds(q0, TQ)].astype(f32) + col(2) * attn
    x1_s[...] = x1
    h2t = _ln_t(x1) * col(4) + col(3)
    h2t = jnp.concatenate([h2t, jnp.zeros((DP - D, TQ), f32)], axis=0)
    h2_s[...] = h2t.T[:, 0:D].astype(bf16)
    acc_s[...] = ffn(0, F0)

    def ffn_body(fi, carry):
        f0 = pl.multiple_of(F0 + fi * FC, 128)
        y = acc_s[...] + ffn(f0, FC)
        acc_s[...] = y
        o_ref[...] = (x1_s[...] + col(5) * y).astype(o_ref.dtype)
        return carry

    lax.fori_loop(0, NF, ffn_body, 0)


@jax.jit
def pallas_adaLN_cond__grouped_kv_mqa__swiglu_ffn__prompt_kernel(
    A_x: jax.Array,
    A_wq: jax.Array,
    A_wk: jax.Array,
    A_wv: jax.Array,
    A_wo: jax.Array,
    B_x: jax.Array,
    B_w_gate: jax.Array,
    B_w_up: jax.Array,
    B_w_down: jax.Array,
    c: jax.Array,
    w_mod: jax.Array,
):
    del B_x
    out_t = pl.pallas_call(
        _kernel,
        grid=(NQ,),
        in_specs=[pl.BlockSpec(memory_space=pltpu.HBM)] * 10,
        out_specs=pl.BlockSpec((D, TQ), lambda i: (0, i)),
        out_shape=jax.ShapeDtypeStruct((D, S), bf16),
        scratch_shapes=[
            pltpu.VMEM((D, S), bf16),
            pltpu.VMEM((D, D), bf16),
            pltpu.VMEM((D, D), bf16),
            pltpu.VMEM((D, 6 * D), bf16),
            pltpu.VMEM((D, F), bf16),
            pltpu.VMEM((D, F), bf16),
            pltpu.VMEM((D, F), bf16),
            pltpu.SemaphoreType.DMA((12,)),
            pltpu.VMEM((6 * D, 128), f32),
            pltpu.VMEM((DP, DP), f32),
            pltpu.VMEM((D, D), bf16),
            pltpu.VMEM((NQ * H, 32, TQ), i32),
            pltpu.VMEM((NQ * H, 8, TQ), i32),
            pltpu.VMEM((HG, S // 4, 128), i32),
            pltpu.VMEM((NQ, 8, 128), i32),
            pltpu.VMEM((VR, S), f32),
            pltpu.VMEM((2, S, TQ), f32),
            pltpu.VMEM((8, TQ), f32),
            pltpu.VMEM((NG, HG * DH, TQ), f32),
            pltpu.VMEM((D, TQ), f32),
            pltpu.VMEM((TQ, D), bf16),
            pltpu.VMEM((D, TQ), f32),
            pltpu.VMEM((2 * VR + D, D), bf16),
            pltpu.VMEM((DH, D), bf16),
            pltpu.VMEM((DH, D), bf16),
            pltpu.VMEM((1, D), bf16),
        ],
        compiler_params=pltpu.CompilerParams(
            dimension_semantics=("arbitrary",),
            vmem_limit_bytes=100 * 1024 * 1024),
    )(c, A_wk.T, A_wv.T, A_x.reshape(S, D).T, A_wq, A_wo, w_mod, B_w_gate, B_w_up, B_w_down.T)
    return out_t.T.reshape(1, S, D)
```

```python
import math

import jax
import jax.numpy as jnp
from jax import lax
import jax.experimental.pallas as pl
import jax.experimental.pallas.tpu as pltpu

f32 = jnp.float32
bf16 = jnp.bfloat16
i32 = jnp.int32
i8 = jnp.int8

S = 2048
D = 576
H = 32
DH = 18
F = 4608
DP = 640
HG = 4
NG = H // HG
VR = 24
EPS = 1e-5
QSCALE = DH ** -0.5 * math.log2(math.e)
NT = (((1,), (1,)), ((), ()))
RND = 1.5 * 2.0 ** 23
T1 = 16.0
T2 = 16.0

TQ = 512
CK = 128
HI = 8
G = 3
SK = 9
TL = 3
F0 = 768
FC = 1280

NQ = S // TQ
NC = S // CK
CPR = TQ // CK
QT = TQ // 128
NTL = NC * QT
TOT = HI * NTL
NF = (F - F0) // FC
assert F0 + NF * FC == F


def _ln_t(x):
    def mean0(v):
        v = v.reshape(D // 16, 16, v.shape[1]).sum(axis=0)
        return jnp.sum(v, axis=0, keepdims=True) * (1.0 / D)

    xc = x - mean0(x)
    return xc * lax.rsqrt(mean0(xc * xc) + EPS)


def _expo(a, lo, hi):
    a = jnp.minimum(jnp.maximum(a, 2.0 ** lo), 2.0 ** hi)
    return lax.bitcast_convert_type(a, i32) & 0x7F800000


def _pow2(bits):
    return lax.bitcast_convert_type(bits, f32)


def _inv2(bits):
    return lax.bitcast_convert_type((254 << 23) - bits, f32)


def _lanes(v, k):
    return v[:, k * 128:(k + 1) * 128]


def _runs(n0, n1):
    out = []
    while n0 < n1:
        hd, r = divmod(n0, NTL)
        c, qt = divmod(r, QT)
        e = min(QT, qt + n1 - n0)
        out.append((hd, c, qt, e))
        n0 += e - qt
    return out


def _b_target(a_done):
    best = 0
    for jb in range(HI):
        lo = 0 if jb == 0 else jb * NTL + SK
        hi = min(lo + NTL, TOT - TL)
        if a_done > lo:
            best = jb * NTL + min(NTL, -(-(a_done - lo) * NTL // (hi - lo)))
    return best


def _kernel(c_hbm, wkt_hbm, wvt_hbm, xt_hbm, wq_hbm, wo_hbm, wmod_hbm, wg_hbm, wu_hbm, wdt_hbm,
            o_ref,
            xt_v, wq_v, wo_v, wmod_v, wg_v, wu_v, wdt_v, sems,
            modt_s, tmp_s, wot_s, q_s, mg_s, k_s, ek_s, vt_s, s_s,
            mn_s, ot_s, x1_s, h2_s, acc_s, wall_s, wkt_v, wvt_v, c_v):
    i = pl.program_id(0)

    def cp_cols(src, dst, lo, hi, k):
        return pltpu.make_async_copy(src.at[:, lo:hi], dst.at[:, lo:hi], sems.at[k])

    cp_mod0 = lambda: cp_cols(wmod_hbm, wmod_v, 0, 2 * D, 0)
    cp_mod1 = lambda: cp_cols(wmod_hbm, wmod_v, 2 * D, 6 * D, 1)
    cp_x0 = lambda: cp_cols(xt_hbm, xt_v, 0, TQ, 2)
    cp_x1 = lambda: cp_cols(xt_hbm, xt_v, TQ, S, 3)
    cp_wo = lambda: pltpu.make_async_copy(wo_hbm, wo_v, sems.at[4])
    cp_first = lambda: [
        pltpu.make_async_copy(src, dst, sems.at[5 + k]) for k, (src, dst) in enumerate(
            ((wq_hbm, wq_v), (wkt_hbm, wkt_v), (wvt_hbm, wvt_v), (c_hbm, c_v)))]
    cp_ffn = lambda: [
        pltpu.make_async_copy(src, dst, sems.at[9 + k]) for k, (src, dst) in enumerate(
            ((wg_hbm, wg_v), (wu_hbm, wu_v), (wdt_hbm, wdt_v)))]

    def mod_cols(lo, hi):
        cc = c_v[...].astype(f32)
        sc = jnp.broadcast_to(cc * (1.0 / (1.0 + jnp.exp(-cc))), (8, D))
        row = jnp.dot(sc, wmod_v[:, lo:hi], preferred_element_type=f32)[0:1]
        lane = lax.broadcasted_iota(i32, (1, hi - lo), 1) + lo
        scale = ((lane >= D) & (lane < 2 * D)) | ((lane >= 4 * D) & (lane < 5 * D))
        row = jnp.where(scale, row + 1.0, row)
        modt_s[lo:hi, :] = jnp.broadcast_to(row, (128, hi - lo)).T

    def col(k):
        return jnp.tile(modt_s[k * D:(k + 1) * D, :], (1, QT))

    def transpose_w(w_v):
        tmp_s[0:D, 0:D] = w_v[...].astype(f32)
        return tmp_s[...].T[0:D, 0:D]

    class Head:
        def __init__(self, h, m=None):
            self.h = h
            self.mgq = mg_s[h]
            self.mg = {}
            self.mb = {}
            self.mt = {}
            self.m = m
            self.off = {}
            self.acc = {}

        def bias_bits(self, qt, r):
            return _lanes(self.mgq, qt) + ek_s[r]

    def a_run(hd, j, c, q0t, q1t, buf):
        if c % CPR == 0:
            for qt in range(q0t, q1t):
                hd.mg[qt] = hd.bias_bits(qt, c // CPR)
        mg = jnp.concatenate([hd.mg[qt] for qt in range(q0t, q1t)], axis=1)
        qd = q_s[hd.h, :, q0t * 128:q1t * 128]
        kd = k_s[j, c * CK:(c + 1) * CK, :]
        n = jnp.dot(kd, qd, preferred_element_type=i32)
        s = lax.bitcast_convert_type(n + jnp.tile(mg, (CK // 8, 1)), f32)
        s_s[buf, c * CK:(c + 1) * CK, q0t * 128:q1t * 128] = s
        mc = s.reshape(CK // 8, 8, (q1t - q0t) * 128).max(axis=0)
        for qt in range(q0t, q1t):
            v = _lanes(mc, qt - q0t)
            hd.mb[qt] = v if c % CPR == 0 else jnp.maximum(hd.mb[qt], v)
            if c % CPR == CPR - 1:
                v = hd.mb[qt] - lax.bitcast_convert_type(hd.mg[qt], f32)
                hd.mt[qt] = v if c < CPR else jnp.maximum(hd.mt[qt], v)
        if c == NC - 1 and q1t == QT:
            m = jnp.concatenate([hd.mt[qt] for qt in range(QT)], axis=1)
            hd.m = jnp.broadcast_to(m.max(axis=0, keepdims=True), (8, TQ))

    def b_run(hd, c, q0t, q1t, buf, g, j):
        sl = slice(c * CK, (c + 1) * CK)
        if c % CPR == 0:
            for qt in range(q0t, q1t):
                hd.off[qt] = _lanes(hd.m, qt) + lax.bitcast_convert_type(hd.bias_bits(qt, c // CPR), f32)
        off = jnp.concatenate([hd.off[qt] for qt in range(q0t, q1t)], axis=1)
        p = jnp.exp2(s_s[buf, sl, q0t * 128:q1t * 128] - jnp.tile(off, (CK // 8, 1)))
        pv = jnp.dot(vt_s[:, sl], p.astype(bf16), preferred_element_type=f32)
        for qt in range(q0t, q1t):
            v = _lanes(pv, qt - q0t)
            acc = hd.acc[qt] = v if c == 0 else hd.acc[qt] + v
            if c == NC - 1:
                ot_s[g, j * DH:(j + 1) * DH, qt * 128:(qt + 1) * 128] = (
                    acc * (1.0 / acc[DH:DH + 1]))[0:DH]

    @pl.when(i == 0)
    def _prologue():
        for cp in cp_first():
            cp.start()
        cp_mod0().start()
        cp_x0().start()
        cp_x1().start()
        cp_wo().start()
        cp_mod1().start()

        tmp_s[:, D:DP] = jnp.zeros((DP, DP - D), f32)
        tmp_s[D:DP, :] = jnp.zeros((DP - D, DP), f32)

        for cp in cp_first():
            cp.wait()
        z6 = jnp.zeros((VR - DH, D), f32)
        wk = jnp.concatenate([wkt_v[...].astype(f32), z6], axis=0)
        wall_s[0:2 * VR, :] = jnp.concatenate([wvt_v[...].astype(f32), z6, wk], axis=0).astype(bf16)
        eb = _expo(jnp.broadcast_to(jnp.max(jnp.abs(wk), axis=1, keepdims=True), (VR, 128)),
                   -60, 60)
        kbal = _inv2(eb) * QSCALE
        qbal = jnp.concatenate([_pow2(eb)[0:DH]] * HG, axis=0)
        qbal = jnp.tile(qbal, (NG, DP // 128))[:, 0:D]
        wall_s[2 * VR:, :] = (transpose_w(wq_v) * qbal).astype(bf16)

        cp_mod0().wait()
        mod_cols(0, 2 * D)

        vrow = lax.broadcasted_iota(i32, (VR, 1), 0)
        row8 = lax.broadcasted_iota(i32, (1, 8, 1), 1)
        clip8 = lambda v: jnp.clip(v, -127.0, 127.0)

        def k_digits(r, kt):
            kt = kt * jnp.tile(kbal, (1, QT))
            kmax = jnp.max(jnp.max(jnp.abs(kt), axis=0, keepdims=True), axis=1, keepdims=True)
            ek = _expo(jnp.broadcast_to(kmax, (8, 128)) * (512.0 / 381.4), -30, 46)
            ek_s[r] = ek - (135 << 23)
            kt = kt * jnp.tile(_inv2(ek) * 256.0, (VR // 8, QT))
            k1 = (kt + RND) - RND
            ka = clip8(k1)
            kb = clip8(k1 - ka)
            kd = jnp.concatenate(
                [ka + RND, kb + RND, (k1 - ka - kb) + RND, kt * (1.0 / T1) + RND,
                 (kt - k1) * T2 + RND, jnp.zeros((8, TQ), f32)], axis=0)
            kd = lax.bitcast_convert_type(kd.T, i32)
            for j in range(HG):
                k_s[j, r * TQ:(r + 1) * TQ, :] = (
                    kd if j == 0 else pltpu.roll(kd, 2 * j, 1)).astype(i8)

        pend = None
        for r in range(NQ):
            if r == 0:
                cp_x0().wait()
            if r == 1:
                cp_x1().wait()
                for cp in cp_ffn():
                    cp.start()
            if r == NQ - 1:
                cp_wo().wait()
                cp_mod1().wait()
            tok = slice(r * TQ, (r + 1) * TQ)
            if pend is not None:
                k_digits(*pend)
                pend = None
            h = (_ln_t(xt_v[:, tok].astype(f32)) * col(1) + col(0)).astype(bf16)
            res = jnp.dot(wall_s[...], h, preferred_element_type=f32)
            if r == NQ - 1:
                wot_s[...] = transpose_w(wo_v).astype(bf16)
            vt_s[:, tok] = jnp.where(vrow == DH, 1.0, res[0:VR])

            if r in (0, NQ - 2):
                pend = (r, res[VR:2 * VR])
            else:
                k_digits(r, res[VR:2 * VR])

            qt = res[2 * VR:].reshape(NG, HG * DH, TQ)
            qa = jnp.abs(qt)
            inv = []
            for j in range(HG):
                w = [qa[:, 16 * j + 8 * t:16 * j + 8 * (t + 1)] for t in range(3)]
                if j > 0:
                    w[0] = jnp.where(row8 >= 2 * j, w[0], 0.0)
                if j < HG - 1:
                    w[2] = jnp.where(row8 < 2 * j + 2, w[2], 0.0)
                amax = jnp.max(jnp.maximum(jnp.maximum(w[0], w[1]), w[2]), axis=1, keepdims=True)
                eq = jnp.broadcast_to(_expo(amax * (2.0 / 127.4), -106, 64), (NG, 8, TQ))
                for g in range(NG):
                    mg_s[r * H + g * HG + j] = eq[g] + ((23 << 23) + 0x400000)
                inv.append(_inv2(eq))
            mix = lambda j: jnp.where(row8 < 2 * j + 2, inv[j], inv[j + 1])
            qt = qt * jnp.concatenate(
                [inv[0], inv[0], mix(0), inv[1], mix(1), inv[2], mix(2), inv[3], inv[3]], axis=1)
            t1 = qt + RND
            b1 = lax.bitcast_convert_type(t1, i32)
            ba = lax.bitcast_convert_type((qt - (t1 - RND)) * T1 + RND, i32)
            bc = lax.bitcast_convert_type(qt * (1.0 / T2) + RND, i32)
            for j in range(HG):
                win = slice(16 * j, 16 * j + VR)
                qd = jnp.concatenate(
                    [b1[:, win], b1[:, win], b1[:, win], ba[:, win], bc[:, win],
                     jnp.zeros((NG, 8, TQ), i32)], axis=1)
                qd = qd.astype(i8)
                for g in range(NG):
                    q_s[r * H + g * HG + j] = qd[g]

        hd = Head(0)
        for c in range(NC):
            a_run(hd, 0, c, 0, QT, 0)
            if c < 9:
                mod_cols(2 * D + 256 * c, 2 * D + 256 * (c + 1))
        mn_s[...] = hd.m

    def attn_body(it, m_next):
        h0 = i * H + it * HI
        g0 = it * (HI // HG)
        hn = jnp.minimum(h0 + HI, NQ * H - HG)
        heads = {0: Head(h0, m_next)}
        a_done = b_done = 0
        while a_done < TOT:
            a1 = min(TOT, a_done + G)
            for ha, c, q0t, q1t in _runs(a_done, a1):
                ja = ha + 1
                if ja not in heads:
                    heads[ja] = Head(h0 + ja if ja < HI else hn)
                a_run(heads[ja], ja % HG, c, q0t, q1t, ja % 2)
            a_done = a1
            b1 = _b_target(a_done)
            for jb, c, q0t, q1t in _runs(b_done, b1):
                b_run(heads[jb], c, q0t, q1t, jb % 2, g0 + jb // HG, jb % HG)
            b_done = b1
        assert b_done == TOT
        return heads[HI].m

    mn_s[...] = lax.fori_loop(0, H // HI, attn_body, mn_s[...])

    @pl.when(i == 0)
    def _():
        for cp in cp_ffn():
            cp.wait()

    def ffn(f0, fc):
        h2 = h2_s[...]
        g = jnp.dot(h2, wg_v[:, pl.ds(f0, fc)], preferred_element_type=f32)
        u = jnp.dot(h2, wu_v[:, pl.ds(f0, fc)], preferred_element_type=f32)
        gh = 0.5 * g
        a = ((gh + gh * jnp.tanh(gh)) * u).astype(bf16)
        return lax.dot_general(wdt_v[:, pl.ds(f0, fc)], a, NT, preferred_element_type=f32)

    q0 = pl.multiple_of(i * TQ, TQ)
    ot = ot_s[...].reshape(D, TQ).astype(bf16)
    attn = jnp.dot(wot_s[...], ot, preferred_element_type=f32)
    x1 = xt_v[:, pl.ds(q0, TQ)].astype(f32) + col(2) * attn
    x1_s[...] = x1
    h2t = _ln_t(x1) * col(4) + col(3)
    h2t = jnp.concatenate([h2t, jnp.zeros((DP - D, TQ), f32)], axis=0)
    h2_s[...] = h2t.T[:, 0:D].astype(bf16)
    acc_s[...] = ffn(0, F0)

    def ffn_body(fi, carry):
        f0 = pl.multiple_of(F0 + fi * FC, 128)
        y = acc_s[...] + ffn(f0, FC)
        acc_s[...] = y
        o_ref[...] = (x1_s[...] + col(5) * y).astype(o_ref.dtype)
        return carry

    lax.fori_loop(0, NF, ffn_body, 0)


@jax.jit
def pallas_adaLN_cond__grouped_kv_mqa__swiglu_ffn__prompt_kernel(
    A_x: jax.Array,
    A_wq: jax.Array,
    A_wk: jax.Array,
    A_wv: jax.Array,
    A_wo: jax.Array,
    B_x: jax.Array,
    B_w_gate: jax.Array,
    B_w_up: jax.Array,
    B_w_down: jax.Array,
    c: jax.Array,
    w_mod: jax.Array,
):
    del B_x
    out_t = pl.pallas_call(
        _kernel,
        grid=(NQ,),
        in_specs=[pl.BlockSpec(memory_space=pltpu.HBM)] * 10,
        out_specs=pl.BlockSpec((D, TQ), lambda i: (0, i)),
        out_shape=jax.ShapeDtypeStruct((D, S), bf16),
        scratch_shapes=[
            pltpu.VMEM((D, S), bf16),
            pltpu.VMEM((D, D), bf16),
            pltpu.VMEM((D, D), bf16),
            pltpu.VMEM((D, 6 * D), bf16),
            pltpu.VMEM((D, F), bf16),
            pltpu.VMEM((D, F), bf16),
            pltpu.VMEM((D, F), bf16),
            pltpu.SemaphoreType.DMA((12,)),
            pltpu.VMEM((6 * D, 128), f32),
            pltpu.VMEM((DP, DP), f32),
            pltpu.VMEM((D, D), bf16),
            pltpu.VMEM((NQ * H, 128, TQ), i8),
            pltpu.VMEM((NQ * H, 8, TQ), i32),
            pltpu.VMEM((HG, S, 128), i8),
            pltpu.VMEM((NQ, 8, 128), i32),
            pltpu.VMEM((VR, S), f32),
            pltpu.VMEM((2, S, TQ), f32),
            pltpu.VMEM((8, TQ), f32),
            pltpu.VMEM((NG, HG * DH, TQ), f32),
            pltpu.VMEM((D, TQ), f32),
            pltpu.VMEM((TQ, D), bf16),
            pltpu.VMEM((D, TQ), f32),
            pltpu.VMEM((2 * VR + D, D), bf16),
            pltpu.VMEM((DH, D), bf16),
            pltpu.VMEM((DH, D), bf16),
            pltpu.VMEM((1, D), bf16),
        ],
        compiler_params=pltpu.CompilerParams(
            dimension_semantics=("arbitrary",),
            vmem_limit_bytes=100 * 1024 * 1024),
    )(c, A_wk.T, A_wv.T, A_x.reshape(S, D).T, A_wq, A_wo, w_mod, B_w_gate, B_w_up, B_w_down.T)
    return out_t.T.reshape(1, S, D)
```
